```python
import os as _os
_os.environ.setdefault('JAX_PLATFORMS', 'cpu')
import jax
import jax.numpy as jnp

def _softmax(x, axis=-1):
    return jax.nn.softmax(x, axis=axis)

def _gelu(x):
    return jax.nn.gelu(x, approximate=True)

def _silu(x):
    return jax.nn.silu(x)

def _sigmoid(x):
    return jax.nn.sigmoid(x)

def _layernorm(x, axis=-1, eps=1e-05):
    m = jnp.mean(x, axis=axis, keepdims=True)
    v = jnp.var(x, axis=axis, keepdims=True)
    return (x - m) / jnp.sqrt(v + eps)

def _scatter_add(tgt, idx, src, axis=0):
    return tgt.at[idx].add(src)

def _segment_sum(src, seg, n):
    return jax.ops.segment_sum(src, seg, n)

class _Rng:

    def __init__(self, key):
        self._k = key

    def _next(self):
        self._k, sub = jax.random.split(self._k)
        return sub

    def normal(self, shape):
        return jax.random.normal(self._next(), shape, dtype=jnp.bfloat16)

    def randint(self, lo, hi, shape):
        return jax.random.randint(self._next(), shape, lo, hi, dtype=jnp.int32)

    def uniform(self, shape, lo=0.0, hi=1.0):
        return jax.random.uniform(self._next(), shape, jnp.bfloat16, lo, hi)

    def permutation(self, n):
        return jax.random.permutation(self._next(), n)
kernel_name = 'gated_mix__grouped_kv_mqa__memory_aug_recurrent_mem_tr__prompt'

def setup_inputs():
    _rng = _Rng(jax.random.key(int.from_bytes(__import__("os").urandom(4), "little")))
    _w = lambda a: (lambda t: t.astype(jnp.bfloat16) if jnp.issubdtype(t.dtype, jnp.floating) else t)(jnp.asarray(a))

    def _A_setup():
        B, S, D, H = (1, 2048, 1024, 32)
        Dh = D // H
        return {'x': _w((lambda *s: _rng.normal(s) * 0.05)(B, S, D)), 'wq': _w((lambda *s: _rng.normal(s) * 1.6)(D, H * Dh)), 'wk': _w((lambda *s: _rng.normal(s) * 1.6)(D, Dh)), 'wv': _w((lambda *s: _rng.normal(s) * 0.05)(D, Dh)), 'wo': _w((lambda *s: _rng.normal(s) * 0.05)(H * Dh, D))}
    _A_in = _A_setup()

    def _B_setup():
        B, S, Dm = (1, 2048, 1024)
        H, Dh = (32, 128)
        M, seg = (8, 32)
        seg = min(seg, S)
        S = S // seg * seg
        return {'x': _w((lambda *s: _rng.normal(s) * 0.05)(B, S, Dm)), 'mem0': _w((lambda *s: _rng.normal(s) * 0.8)(B, M, Dm)), 'Wq': _w((lambda *s: _rng.normal(s) * 3.2)(Dm, H, Dh) * Dm ** (-0.5)), 'Wk': _w((lambda *s: _rng.normal(s) * 3.2)(Dm, H, Dh) * Dm ** (-0.5)), 'Wv': _w((lambda *s: _rng.normal(s) * 0.8)(Dm, H, Dh) * Dm ** (-0.5)), 'Wo': _w((lambda *s: _rng.normal(s) * 0.8)(H, Dh, Dm) * (H * Dh) ** (-0.5)), 'seg_len': seg}
    _B_in = _B_setup()
    return {'A_x': _A_in['x'], 'A_wq': _A_in['wq'], 'A_wk': _A_in['wk'], 'A_wv': _A_in['wv'], 'A_wo': _A_in['wo'], 'B_x': _B_in['x'], 'B_mem0': _B_in['mem0'], 'B_Wq': _B_in['Wq'], 'B_Wk': _B_in['Wk'], 'B_Wv': _B_in['Wv'], 'B_Wo': _B_in['Wo'], 'B_seg_len': _B_in['seg_len'], 'gate_w': _w((lambda *s: _rng.normal(s) * 0.05)(1024) * 16.0)}

def reference(A_x, A_wq, A_wk, A_wv, A_wo, B_x, B_mem0, B_Wq, B_Wk, B_Wv, B_Wo, B_seg_len, gate_w):

    def _A_ref(x, wq, wk, wv, wo):
        B, S, D = x.shape
        H = 32
        Dh = D // H
        q = (lambda x, *d: x.transpose(*d))((x @ wq).reshape(B, S, H, Dh), 0, 2, 1, 3)
        k = x @ wk
        v = x @ wv
        scores = jnp.einsum('bhqd,bkd->bhqk', q, k) * Dh ** (-0.5)
        p = _softmax(scores, axis=-1)
        o = jnp.einsum('bhqk,bkd->bhqd', p, v)
        return (lambda x, *d: x.transpose(*d))(o, 0, 2, 1, 3).reshape(B, S, H * Dh) @ wo

    def _B_ref(x, mem0, Wq, Wk, Wv, Wo, seg_len):
        B, S, Dm = x.shape
        H, Dh = (Wq.shape[1], Wq.shape[2])
        M = mem0.shape[1]
        scale = Dh ** (-0.5)
        n_seg = S // seg_len
        L = M + seg_len
        idx = jnp.arange(L)
        mask = (idx[:, None] < M) | (idx[:, None] >= idx[None, :])
        mem = mem0
        outs = []
        for s in range(n_seg):
            xs = x[:, s * seg_len:(s + 1) * seg_len, :].copy()
            h = jnp.concatenate([mem, xs], axis=1)
            q = jnp.einsum('btd,dhe->bhte', h, Wq)
            k = jnp.einsum('btd,dhe->bhte', h, Wk)
            v = jnp.einsum('btd,dhe->bhte', h, Wv)
            scores = jnp.einsum('bhqe,bhke->bhqk', q, k) * scale
            scores = jnp.where(mask[None, None], scores, -1000000000.0)
            p = _softmax(scores, axis=-1)
            o = jnp.einsum('bhqk,bhke->bhqe', p, v)
            o = jnp.einsum('bhte,hed->btd', o, Wo)
            mem = o[:, :M, :].copy()
            outs.append(o[:, M:, :])
        return jnp.concatenate(outs, axis=1)
    x = A_x
    g = _sigmoid((x * gate_w).sum(-1, keepdims=True))
    a = _A_ref(x, A_wq, A_wk, A_wv, A_wo)
    b = _B_ref(x, B_mem0, B_Wq, B_Wk, B_Wv, B_Wo, B_seg_len)
    return g * a + (1 - g) * b
```

```python
import functools

import jax
import jax.numpy as jnp
import jax.experimental.pallas as pl
import jax.experimental.pallas.tpu as pltpu

bf16 = jnp.bfloat16
f32 = jnp.float32
u32 = jnp.uint32

S = 2048
D = 1024
H = 32
DHA = 32
DHB = 128
M = 8
SEG = 32
L = M + SEG
LOG2E = 1.4426950408889634
CA = DHA ** -0.5 * LOG2E
CB = DHB ** -0.5 * LOG2E

XCH = 4
XR = S // XCH
QB = 512
CK = 128
NC = S // CK
NGA = (S // QB) * 8
LAG = 2
PACE = 2
WCH = 8
WR = D // WCH
GB = 3
SP = 40

NT = (((1,), (1,)), ((), ()))


def _kernel(x_hbm, wq_hbm, wkt_ref, wvt_ref, wo_hbm, mem0_ref, bq_hbm, bk_hbm, bv_hbm, bo_hbm, gate_ref,
            out_hbm,
            x_v, wq_v, wo_v, stage_v, w_v, bo_v, q_v, kp_v, vt_v, s0, s1, s2, s3, ot_v, mx_v, m3_v, l_v,
            o_v, mem_v, out_v, z_ref, sem_x, sem_w, sem_b, sem_bo, sem_o):
    cp_wq = pltpu.make_async_copy(wq_hbm, wq_v, sem_w)
    cp_wq.start()
    for i in range(XCH):
        pltpu.make_async_copy(x_hbm.at[pl.ds(i * XR, XR)], x_v.at[pl.ds(i * XR, XR)], sem_x.at[i]).start()

    def cp_b(c):
        r0 = pl.multiple_of(c * WR, WR)
        return [pltpu.make_async_copy(src.at[pl.ds(r0, WR)], stage_v.at[t, pl.ds(r0, WR)], sem_b.at[c])
                for t, src in enumerate((bq_hbm, bk_hbm, bv_hbm))]

    cp_bo = [pltpu.make_async_copy(bo_hbm.at[:, pl.ds(j * 128, 128)], bo_v.at[j], sem_bo)
             for j in range(8)]
    cp_bo += [pltpu.make_async_copy(wo_hbm.at[:, pl.ds(j * 128, 128)], wo_v.at[j], sem_bo)
              for j in range(8)]

    z_ref[0] = 0
    z_ref[1] = 0

    wkvt = jnp.concatenate([wkt_ref[...], wvt_ref[...]], axis=0)
    lane_grp = jax.lax.broadcasted_iota(jnp.int32, (XR, 128), 1) // DHA
    cp_wq.wait()

    def a_proj(i, carry):
        r0 = pl.multiple_of(i * XR, XR)
        pltpu.make_async_copy(x_hbm.at[pl.ds(r0, XR)], x_v.at[pl.ds(r0, XR)], sem_x.at[i]).wait()

        @pl.when(i == XCH - 1)
        def _():
            for c in cp_b(0) + cp_b(1):
                c.start()

        xc = x_v[pl.ds(r0, XR), :]
        kvt = jax.lax.dot_general(wkvt, xc, NT, preferred_element_type=f32)
        vt_v[:, pl.ds(r0, XR)] = kvt[DHA:].astype(bf16)
        k4 = jnp.concatenate([kvt[:DHA]] * 4, axis=0).T
        for j in range(4):
            kp_v[j, pl.ds(r0, XR), :] = jnp.where(lane_grp == j, k4, 0.0).astype(bf16)
        for g in range(8):
            qg = jnp.dot(xc, wq_v[:, g * 128:(g + 1) * 128], preferred_element_type=f32) * CA
            q_v[g, pl.ds(r0, XR), :] = qg.astype(bf16)
        return carry

    jax.lax.fori_loop(0, XCH, a_proj, 0)

    bufs = (s0, s1, s2, s3)

    def load_q(it):
        qb = jax.lax.shift_right_logical(it, 3)
        g = it & 7
        return q_v[g, pl.ds(pl.multiple_of(qb * QB, QB), QB), :]

    def p1chunk(qg, j, c, mx, z):
        k = kp_v[j, c * CK:(c + 1) * CK, :]
        s = jax.lax.dot_general(k, qg, NT, preferred_element_type=f32)
        bufs[j][pl.ds(pl.multiple_of(z + c * CK, 8), CK), :] = s
        sm = jnp.max(s.reshape(CK // 8, 8, QB), axis=0)
        return sm if mx is None else jnp.maximum(mx, sm)

    def p2chunk(j, m, c, l, o, z):
        sc = bufs[j][pl.ds(pl.multiple_of(z + c * CK, 8), CK), :].reshape(CK // 8, 8, QB)
        p = jnp.exp2(sc - m[None])
        t = p
        while t.shape[0] > 1:
            t4 = t.reshape(t.shape[0] // 2, 2, 8, QB)
            t = t4[:, 0] + t4[:, 1]
        ls = t[0]
        l = ls if l is None else l + ls
        pb = p.reshape(CK, QB).astype(bf16)
        oc = jnp.dot(vt_v[:, c * CK:(c + 1) * CK], pb, preferred_element_type=f32)
        return l, (oc if o is None else oc + o)

    def colmax(mx):
        return jnp.broadcast_to(jnp.max(mx, axis=0, keepdims=True), (8, QB))

    def fin(it, l3, o3):
        qb = jax.lax.shift_right_logical(it, 3)
        g = it & 7
        parts = []
        for j in range(4):
            lj = l_v[j * 8:(j + 1) * 8, :] if j < 3 else l3
            oj = ot_v[j * 32:(j + 1) * 32, :] if j < 3 else o3
            parts.append(oj * pl.reciprocal(jnp.sum(lj, axis=0, keepdims=True), approx=False))
        ot = jnp.concatenate(parts, axis=0)
        o_v[g, pl.ds(pl.multiple_of(qb * QB, QB), QB), :] = ot.T.astype(bf16)

    def relayout(t, b, hq):
        blk = stage_v[t, pl.ds(pl.multiple_of(b * 16, 16), 16), hq * 8:(hq + 1) * 8, :]
        w_v[t, hq * 8:(hq + 1) * 8, pl.ds(pl.multiple_of(b * 8, 8), 8), :] = pltpu.bitcast(
            jnp.swapaxes(blk, 0, 1), u32)

    ot_v[...] = jnp.zeros_like(ot_v)
    l_v[...] = jnp.ones_like(l_v)
    m3_v[...] = jnp.zeros_like(m3_v)
    s3[(NC - LAG) * CK:, :] = jnp.zeros((LAG * CK, QB), f32)
    qg0 = load_q(0)
    mx0 = None
    for c in range(NC):
        mx0 = p1chunk(qg0, 0, c, mx0, z_ref[0])
    mx_v[...] = mx0

    def a_body(it, carry):
        @pl.when((it & 3) == 0)
        def _():
            ch = jax.lax.shift_right_logical(it, 2)
            for c in cp_b(ch):
                c.wait()

            @pl.when(ch < WCH - 2)
            def _():
                for c in cp_b(ch + 2):
                    c.start()

            @pl.when(ch == WCH - 2)
            def _():
                for c in cp_bo:
                    c.start()

        zs = z_ref[0]
        zl = z_ref[1]
        qg = load_q(it)
        qgn = load_q(jnp.minimum(it + 1, NGA - 1))
        mxs = {0: mx_v[...]}
        ms = {-1: m3_v[...]}
        l = l_v[24:32, :]
        o = ot_v[96:128, :]
        mx = None
        hist = []
        for t in range(4 * NC):
            j1, c1 = t // NC + 1, t % NC
            mx = p1chunk(qg if j1 < 4 else qgn, j1 % 4, c1, None if c1 == 0 else mx, zs)
            hist.append(mx)
            if c1 == NC - 1:
                mxs[j1] = mx
            j2, c2 = divmod(t - LAG, NC)
            if c2 == 0:
                ms[j2] = colmax(mxs[j2])
                l = o = None
            mm = ms[j2]
            if t >= PACE:
                mm = jnp.maximum(mm, hist[t - PACE] - jnp.inf)
            l, o = p2chunk(j2 % 4, mm, c2, l, o, zl)
            if c2 == NC - 1:
                if j2 < 0:
                    fin(jnp.maximum(it - 1, 0), l, o)
                else:
                    ot_v[j2 * 32:(j2 + 1) * 32, :] = o
                    l_v[j2 * 8:(j2 + 1) * 8, :] = l
            if 8 <= t < 56 and t % 2 == 0:
                k = (t - 8) // 2
                relayout(k // 8, it * 2 + (k // 4) % 2, k % 4)
        ot_v[96:128, :] = o
        l_v[24:32, :] = l
        m3_v[...] = ms[3]
        mx_v[...] = mx
        return carry

    jax.lax.fori_loop(0, NGA, a_body, 0)
    l = l_v[24:32, :]
    o = ot_v[96:128, :]
    for c in range(NC - LAG, NC):
        l, o = p2chunk(3, m3_v[...], c, l, o, z_ref[1])
    fin(NGA - 1, l, o)

    for c in cp_bo:
        c.wait()

    kk = jax.lax.broadcasted_iota(jnp.int32, (L, 128), 0)
    qq = jax.lax.broadcasted_iota(jnp.int32, (L, 128), 1) % SP
    mask = (qq < M) | (qq >= kk)
    gate = gate_ref[...].astype(f32)
    mem_v[...] = mem0_ref[...].astype(f32)
    NGB = -(-H // GB)

    def heads(g):
        return list(range(g * GB, min((g + 1) * GB, H)))

    def step(lhs, regroup, wo_rows, z):
        qkv, pr, ov = {}, {}, {}

        def proj(g):
            for h in heads(g):
                q, k, v = (regroup(h, t, jnp.dot(lhs, pltpu.bitcast(w_v[t + z, h], bf16),
                                                 preferred_element_type=f32))
                           for t in range(3))
                zero8 = jnp.zeros((8, 128), f32)
                qkv[h] = (q * CB, jnp.concatenate([k, zero8], axis=0).astype(bf16),
                          jnp.concatenate([v, zero8], axis=0).astype(bf16))

        def scores(g):
            hs = heads(g)
            st = None
            for i, h in enumerate(hs):
                q, k, _ = qkv[h]
                parts = []
                if i:
                    parts.append(jnp.zeros((i * SP, 128), f32))
                parts.append(q)
                parts.append(jnp.zeros((128 - (i + 1) * SP, 128), f32))
                qp = jnp.concatenate(parts, axis=0).astype(bf16)
                sh = jax.lax.dot_general(k, qp, NT, preferred_element_type=f32)[0:L]
                st = sh if st is None else sh + st
            st = jnp.where(mask, st, -1e9)
            m = jnp.max(st, axis=0, keepdims=True)
            p = jnp.exp2(st - m)
            p = p * pl.reciprocal(jnp.sum(p, axis=0, keepdims=True), approx=False)
            pt = jnp.concatenate([p, jnp.zeros((128 - L, 128), f32)], axis=0).T
            for i, h in enumerate(hs):
                rows = jnp.concatenate([pt[i * SP:(i + 1) * SP], jnp.zeros((8, 128), f32)], axis=0)
                pr[h] = rows[:, 0:48].astype(bf16)

        def pv(g):
            for h in heads(g):
                o = jnp.dot(pr[h], qkv[h][2], preferred_element_type=f32)[0:L]
                ov[h] = wo_rows(h, o).astype(bf16)

        acc = [None] * 8

        def oproj(g4):
            og = jnp.concatenate([ov[h] for h in range(4 * g4, 4 * g4 + 4)], axis=1)
            for j in range(8):
                a = jnp.dot(og, bo_v[j + z, g4 * 512:(g4 + 1) * 512, :], preferred_element_type=f32)
                acc[j] = a if acc[j] is None else a + acc[j]

        for t in range(NGB):
            proj(t)
            if t >= 1:
                scores(t - 1)
            if t >= 2:
                pv(t - 2)
        oproj(0)
        scores(NGB - 1)
        oproj(1)
        pv(NGB - 2)
        oproj(2)
        oproj(3)
        pv(NGB - 1)
        for g4 in range(4, 8):
            oproj(g4)
        return jnp.concatenate(acc, axis=1)

    def b_body(j, carry):
        base = pl.multiple_of(j * 64, 64)
        xa = x_v[pl.ds(base, 32), :]
        xb = x_v[pl.ds(base + 32, 32), :]
        xb32 = xb.astype(f32)
        saved_qkv, saved_o = {}, {}

        lhs_a = jnp.concatenate(
            [xa, jnp.concatenate([mem_v[...], xb32[0:8]], axis=0).astype(bf16)], axis=0)

        def regroup_a(h, t, y):
            saved_qkv[(h, t)] = y[40:48]
            return jnp.concatenate([y[32:40], y[0:32]], axis=0)

        def wo_rows_a(h, o):
            saved_o[h] = o[32:40]
            return o[0:32]

        acc_a = step(lhs_a, regroup_a, wo_rows_a, 0)

        oa = jnp.concatenate([o_v[g, pl.ds(base, 64), :] for g in range(8)], axis=1)
        a_out = jnp.concatenate(
            [jnp.dot(oa, wo_v[c], preferred_element_type=f32) for c in range(8)], axis=1)

        lhs_b = jnp.concatenate(
            [xb[16:32], jnp.concatenate([acc_a[0:8], xb32[8:16]], axis=0).astype(bf16)], axis=0)

        def regroup_b(h, t, y):
            return jnp.concatenate([y[16:24], saved_qkv[(h, t)], y[24:32], y[0:16]], axis=0)

        def wo_rows_b(h, o):
            return jnp.concatenate([o, saved_o[h]], axis=0)

        acc_b = step(lhs_b, regroup_b, wo_rows_b, z_ref[0])
        mem_v[...] = acc_b[0:8]

        b_out = jnp.concatenate([acc_a[8:32], acc_b[40:48], acc_b[8:40]], axis=0)
        x32 = jnp.concatenate([xa.astype(f32), xb32], axis=0)
        g = jax.nn.sigmoid(jnp.sum(x32 * gate, axis=1, keepdims=True))
        out_v[pl.ds(base, 64), :] = (g * a_out + (1.0 - g) * b_out).astype(bf16)
        pltpu.make_async_copy(out_v.at[pl.ds(base, 64)], out_hbm.at[pl.ds(base, 64)], sem_o).start()
        return carry

    jax.lax.fori_loop(0, S // 64, b_body, 0)
    pltpu.make_async_copy(out_v, out_hbm, sem_o).wait()


@functools.partial(jax.jit, static_argnames=("B_seg_len",))
def pallas_gated_mix__grouped_kv_mqa__memory_aug_recurrent_mem_tr__prompt_kernel(
    A_x, A_wq, A_wk, A_wv, A_wo, B_x, B_mem0, B_Wq, B_Wk, B_Wv, B_Wo, B_seg_len, gate_w,
):
    del B_x
    assert B_seg_len == SEG
    assert A_x.shape == (1, S, D) and B_Wq.shape == (D, H, DHB) and B_mem0.shape == (1, M, D)
    any_spec = pl.BlockSpec(memory_space=pl.ANY)
    vmem_spec = pl.BlockSpec(memory_space=pltpu.VMEM)
    out = pl.pallas_call(
        _kernel,
        out_shape=jax.ShapeDtypeStruct((S, D), bf16),
        in_specs=[any_spec, any_spec, vmem_spec, vmem_spec, any_spec, vmem_spec,
                  any_spec, any_spec, any_spec, any_spec, vmem_spec],
        out_specs=any_spec,
        scratch_shapes=[
            pltpu.VMEM((S, D), bf16),
            pltpu.VMEM((D, D), bf16),
            pltpu.VMEM((8, D, 128), bf16),
            pltpu.VMEM((3, D, H, DHB), bf16),
            pltpu.VMEM((3, H, D // 2, DHB), u32),
            pltpu.VMEM((8, H * DHB, 128), bf16),
            pltpu.VMEM((8, S, 128), bf16),
            pltpu.VMEM((4, S, 128), bf16),
            pltpu.VMEM((DHA, S), bf16),
            pltpu.VMEM((S, QB), f32),
            pltpu.VMEM((S, QB), f32),
            pltpu.VMEM((S, QB), f32),
            pltpu.VMEM((S, QB), f32),
            pltpu.VMEM((128, QB), f32),
            pltpu.VMEM((8, QB), f32),
            pltpu.VMEM((8, QB), f32),
            pltpu.VMEM((32, QB), f32),
            pltpu.VMEM((8, S, 128), bf16),
            pltpu.VMEM((M, D), f32),
            pltpu.VMEM((S, D), bf16),
            pltpu.SMEM((2,), jnp.int32),
            pltpu.SemaphoreType.DMA((XCH,)),
            pltpu.SemaphoreType.DMA,
            pltpu.SemaphoreType.DMA((WCH,)),
            pltpu.SemaphoreType.DMA,
            pltpu.SemaphoreType.DMA,
        ],
        compiler_params=pltpu.CompilerParams(vmem_limit_bytes=120 * 1024 * 1024),
    )(
        A_x.reshape(S, D), A_wq, A_wk.T, A_wv.T, A_wo, B_mem0.reshape(M, D),
        B_Wq, B_Wk, B_Wv, B_Wo.reshape(H * DHB, D), gate_w.reshape(1, D),
    )
    return out.reshape(1, S, D)
```

```python
import functools

import jax
import jax.numpy as jnp
import jax.experimental.pallas as pl
import jax.experimental.pallas.tpu as pltpu

bf16 = jnp.bfloat16
f32 = jnp.float32
u32 = jnp.uint32

S = 2048
D = 1024
H = 32
DHA = 32
DHB = 128
M = 8
SEG = 32
L = M + SEG
LP = 48
LOG2E = 1.4426950408889634
CA = DHA ** -0.5 * LOG2E
CB = DHB ** -0.5 * LOG2E

XR = 512
HX = XR // 2
QB = 512
CK = 128
NC = S // CK
NGA = (S // QB) * 8
AU = 2
LAG = 2
PACE = 2
WCH = 8
WR = D // WCH
GB = 2
NGB = H // GB

NT = (((1,), (1,)), ((), ()))


def pack(v):
    return pltpu.bitcast(v.astype(bf16), u32)


def unpack(w):
    return pltpu.bitcast(w, bf16)


def half(r0):
    return r0 // 2 if isinstance(r0, int) else pl.multiple_of(jax.lax.shift_right_logical(r0, 1), 8)


def recip(l):
    r = pl.reciprocal(l, approx=True)
    return r * (2.0 - l * r)


def zero_after(v):
    return (pltpu.bitcast(v, u32) >> 31) >> 1


def _kernel(x_hbm, wq_hbm, wkt_hbm, wvt_hbm, wo_hbm, mem0_hbm, bq_hbm, bk_hbm, bv_hbm, bo_hbm, gate_hbm,
            out_hbm,
            wkv_v, mem0_v, gate_v, x_v, wq_v, wos_v, wo_v, stage_v, w_v, bos_v, bo_v,
            q_v, qn_v, q7_v, kt_v, kp_v, o_v, vt_v, s0, s1, s2, s3, ot_v, mx_v, m3_v, l_v,
            mem_v, out_v, z_ref, sem_x, sem_w, sem_b, sem_s, sem_o):
    def cp_x(r0, n, k):
        return pltpu.make_async_copy(x_hbm.at[pl.ds(r0, n)], x_v.at[pl.ds(r0, n)], sem_x.at[k])

    def cp_wq(k):
        col = k * 256 if isinstance(k, int) else pl.multiple_of(k * 256, 256)
        return pltpu.make_async_copy(wq_hbm.at[:, pl.ds(col, 256)], wq_v.at[k], sem_w.at[k])

    def cp_b(c):
        r0 = pl.multiple_of(c * WR, WR)
        col = pl.multiple_of(c * 128, 128)
        cps = [pltpu.make_async_copy(src.at[pl.ds(r0, WR)], stage_v.at[t, pl.ds(r0, WR)], sem_b.at[c])
               for t, src in enumerate((bq_hbm, bk_hbm, bv_hbm))]
        cps.append(pltpu.make_async_copy(bo_hbm.at[:, pl.ds(col, 128)], bos_v.at[c], sem_b.at[c]))
        cps.append(pltpu.make_async_copy(wo_hbm.at[:, pl.ds(col, 128)], wos_v.at[c], sem_b.at[c]))
        return cps

    cp_kv = [pltpu.make_async_copy(src, wkv_v.at[pl.ds(i * DHA, DHA)], sem_s.at[0])
             for i, src in enumerate((wkt_hbm, wvt_hbm))]
    cp_late = [pltpu.make_async_copy(mem0_hbm, mem0_v, sem_s.at[1]),
               pltpu.make_async_copy(gate_hbm, gate_v, sem_s.at[1])]
    issue = [cp_kv + [cp_x(0, HX, 0)], [cp_wq(0)], [cp_wq(1)], [cp_x(HX, HX, 1)]]

    def start(cps):
        for c in cps:
            c.start()

    def issue_body(i, carry):
        for k, group in enumerate(issue):
            pl.when(i == k)(functools.partial(start, group))
        return carry

    jax.lax.fori_loop(0, len(issue), issue_body, 0)

    for i in range(3):
        z_ref[i] = 0

    def kv_dot(r0, n):
        kvt = jax.lax.dot_general(wkv_v[...], x_v[pl.ds(r0, n), :], NT, preferred_element_type=f32)
        vt_v[:, pl.ds(r0, n)] = pack(kvt[DHA:])
        kt_v[:, pl.ds(r0, n)] = kvt[:DHA]

    def k_pad(r0, n):
        k4 = jnp.concatenate([kt_v[:, pl.ds(r0, n)]] * 4, axis=0).T
        lane_grp = jax.lax.broadcasted_iota(jnp.int32, (n, 128), 1) // DHA
        for j in range(4):
            kp_v[j, pl.ds(half(r0), n // 2), :] = pack(jnp.where(lane_grp == j, k4, 0.0))

    def q_dot(r0, n, k, gg):
        w = wq_v[k, :, gg * 128:(gg + 1) * 128]
        return jnp.dot(x_v[pl.ds(r0, n), :], w, preferred_element_type=f32) * CA

    def q_early(r0, n, k):
        for gg in range(2):
            qn_v[2 * k + gg, pl.ds(r0, n), :] = q_dot(r0, n, k, gg)

    for c in cp_kv:
        c.wait()
    cp_x(0, HX, 0).wait()
    start([cp_wq(2), cp_wq(3)])
    kv_dot(0, HX)

    def early_a(k, carry):
        cp_wq(k).wait()
        cp_x(pl.multiple_of(XR + k * XR, XR), XR, 2 + k).start()
        q_early(0, HX, k)
        return carry

    jax.lax.fori_loop(0, 2, early_a, 0)
    cp_x(HX, HX, 1).wait()
    start([cp_x(3 * XR, XR, 4)])
    kv_dot(HX, HX)
    q_early(HX, HX, 0)
    q_early(HX, HX, 1)
    start(cp_b(0) + cp_late)

    def early_b(k, carry):
        cp_wq(k).wait()
        q_early(0, XR, k)
        return carry

    jax.lax.fori_loop(2, 4, early_b, 0)
    q7_v[...] = jnp.zeros_like(q7_v)

    def a_proj(i, carry):
        r0 = pl.multiple_of(i * XR, XR)
        cp_x(r0, XR, 1 + i).wait()
        kv_dot(r0, XR)
        for g in range(8):
            qg = q_dot(r0, XR, g // 2, g % 2)
            if g < 7:
                q_v[g, :, pl.ds(r0, XR)] = pack(qg.T)
            else:
                q7_v[...] = qg
            if g == 0:
                q_v[7, :, pl.ds(pl.multiple_of(jnp.maximum(r0 - XR, XR), XR), XR)] = pack(q7_v[...].T)
            if 1 <= g <= 3:
                gl = jnp.minimum(3 * (i - 1) + g - 1, 7)
                q_v[gl, :, 0:XR] = pack(qn_v[gl].T)
            if g == 4:
                k_pad(pl.multiple_of(r0 - XR, XR), XR)
            if g == 5:
                k_pad(r0, XR)
        return carry

    jax.lax.fori_loop(1, S // XR, a_proj, 0)
    q_v[7, :, S - XR:] = pack(q7_v[...].T)
    for c in range(1, WCH):
        start(cp_b(c))

    bufs = (s0, s1, s2, s3)
    mid = []

    def load_q(it, last=False):
        qb = jnp.where(last, 0, jax.lax.shift_right_logical(it, 3))
        g = jnp.where(last, 8, it & 7)
        return unpack(q_v[g, :, pl.ds(pl.multiple_of(qb * QB, QB), QB)])

    def p1chunk(qg, j, c, mx, z, zk=0):
        k = unpack(kp_v[j + zk, c * CK // 2:(c + 1) * CK // 2, :])
        s = jnp.dot(k, qg, preferred_element_type=f32)
        bufs[j][pl.ds(pl.multiple_of(z + c * CK, 8), CK), :] = s
        mid.append(s[64:72, QB - 128:])
        sm = jnp.max(s.reshape(CK // 8, 8, QB), axis=0)
        return sm if mx is None else jnp.maximum(mx, sm)

    def p2chunk(j, m, c, l, o, z):
        sc = bufs[j][pl.ds(pl.multiple_of(z + c * CK, 8), CK), :].reshape(CK // 8, 8, QB)
        p = jnp.exp2(sc - m[None])
        t = p
        while t.shape[0] > 1:
            t4 = t.reshape(t.shape[0] // 2, 2, 8, QB)
            t = t4[:, 0] + t4[:, 1]
        ls = t[0]
        l = ls if l is None else l + ls
        pb = p.reshape(CK, QB).astype(bf16)
        oc = jnp.dot(unpack(vt_v[:, c * CK:(c + 1) * CK]), pb, preferred_element_type=f32)
        return l, (oc if o is None else oc + o)

    def colmax(mx):
        return jnp.broadcast_to(jnp.max(mx, axis=0, keepdims=True), (8, QB))

    def fin(it, l3, o3):
        qb = jax.lax.shift_right_logical(it, 3)
        g = it & 7
        parts = []
        for j in range(4):
            lj = l_v[j * 8:(j + 1) * 8, :] if j < 3 else l3
            oj = ot_v[j * 32:(j + 1) * 32, :] if j < 3 else o3
            parts.append(oj * recip(jnp.sum(lj, axis=0, keepdims=True)))
        ot = jnp.concatenate(parts, axis=0)
        o_v[g, pl.ds(pl.multiple_of(qb * (QB // 2), QB // 2), QB // 2), :] = pack(ot.T)

    def relayout(t, b, hq, pace):
        blk = stage_v[t, pl.ds(pl.multiple_of(b * 16, 16), 16), hq * 8:(hq + 1) * 8, :]
        blk = unpack(pltpu.bitcast(blk, u32) | pace[None, 0:4])
        w_v[t, hq * 8:(hq + 1) * 8, pl.ds(pl.multiple_of(b * 8, 8), 8), :] = pltpu.bitcast(
            jnp.swapaxes(blk, 0, 1), u32)

    def repack(src, dst, c, r0, n, pace):
        w = pltpu.bitcast(src[c, pl.ds(pl.multiple_of(r0, 16), n), :], u32).reshape(n // 16, 8, 128)
        dst[c, pl.ds(half(r0), n // 2), :] = (w | pace[None]).reshape(n // 2, 128)

    ot_v[...] = jnp.zeros_like(ot_v)
    l_v[...] = jnp.ones_like(l_v)
    m3_v[...] = jnp.zeros_like(m3_v)
    s3[(NC - LAG) * CK:, :] = jnp.zeros((LAG * CK, QB), f32)
    qg0 = load_q(0)
    mx0 = None
    for c in range(NC):
        mx0 = p1chunk(qg0, 0, c, mx0, z_ref[0])
    mx_v[...] = mx0

    def a_body(i, carry):
        it0 = i * AU
        zz = [z_ref[n] for n in range(3)]
        last = it0 + AU == NGA
        qgs = [load_q(it0 + u) for u in range(AU)] + [load_q(it0 + AU, last)]
        mxs = {0: mx_v[...]}
        ms = {-1: m3_v[...]}
        l = l_v[24:32, :]
        o = ot_v[96:128, :]
        mx = None
        hist = []
        for tt in range(AU * 4 * NC):
            u, t = divmod(tt, 4 * NC)
            it = it0 + u
            j1, c1 = tt // NC + 1, tt % NC
            mx = p1chunk(qgs[j1 // 4], j1 % 4, c1, None if c1 == 0 else mx, zz[0],
                         jnp.where(last, 4, 0) if j1 == 4 * AU else 0 if j1 <= 4 else zz[2])
            hist.append(mx)
            if c1 == NC - 1:
                mxs[j1] = mx
            j2, c2 = divmod(tt - LAG, NC)
            if c2 == 0:
                ms[j2] = colmax(mxs[j2])
                l = o = None
            mm = ms[j2]
            if tt >= PACE:
                mm = pltpu.bitcast(pltpu.bitcast(mm, u32) | zero_after(hist[tt - PACE]), f32)
            l, o = p2chunk(j2 % 4, mm, c2, l, o, zz[1])
            if c2 == NC - 1:
                if j2 % 4 == 3:
                    fin(jnp.maximum(it - 1, 0), l, o)
                else:
                    ot_v[(j2 % 4) * 32:(j2 % 4 + 1) * 32, :] = o
                    l_v[(j2 % 4) * 8:(j2 % 4 + 1) * 8, :] = l
            if 8 <= t < 56:
                pace = zero_after(mid[-2])
                k = (t - 8) // 2
                ch = jax.lax.shift_right_logical(it, 2)
                if t % 2 == 0:
                    relayout(k // 8, it * 2 + (k // 4) % 2, k % 4, pace)
                elif k < 4:
                    repack(bos_v, bo_v, ch, (it & 3) * 1024 + k * 256, 256, pace)
                elif k == 4:
                    repack(wos_v, wo_v, ch, (it & 3) * 256, 256, pace)
        ot_v[96:128, :] = o
        l_v[24:32, :] = l
        m3_v[...] = ms[4 * AU - 1]
        mx_v[...] = mx
        return carry

    def a_outer(ch, carry):
        for c in cp_b(ch):
            c.wait()

        @pl.when(ch == WCH - 1)
        def _():
            kp_v[4] = o_v[0]
            for c in range(4):
                q_v[8, :, c * 128:(c + 1) * 128] = wo_v[c, 0:64, :]

        per = NGA // WCH // AU
        return jax.lax.fori_loop(ch * per, (ch + 1) * per, a_body, carry)

    jax.lax.fori_loop(0, WCH, a_outer, 0)
    l = l_v[24:32, :]
    o = ot_v[96:128, :]
    for c in range(NC - LAG, NC):
        l, o = p2chunk(3, m3_v[...], c, l, o, z_ref[1])
    fin(NGA - 1, l, o)

    qq = jax.lax.broadcasted_iota(jnp.int32, (32, LP), 0)
    kk = jax.lax.broadcasted_iota(jnp.int32, (32, LP), 1)
    mask_a = kk <= jnp.where(qq < M, L - 1, qq)
    qq = jax.lax.broadcasted_iota(jnp.int32, (LP, 2 * LP), 0)
    kk = jax.lax.broadcasted_iota(jnp.int32, (LP, 2 * LP), 1)
    lo = jnp.where(qq < L, 0, LP)
    hi = jnp.where(qq < M, L - 1, jnp.where(qq < L, qq, qq - M + LP))
    mask_b = (kk >= lo) & (kk <= hi)
    for c in cp_late:
        c.wait()
    gate = gate_v[...].astype(f32).reshape(1, D)
    mem_v[...] = mem0_v[...].astype(f32)

    def step(lhs, operands, mask, z):
        qkv, pr, ov = {}, {}, {}

        def proj(g):
            for h in range(g * GB, (g + 1) * GB):
                qkv[h] = operands(h, *(jnp.dot(lhs, unpack(w_v[t + z, h]), preferred_element_type=f32)
                                       for t in range(3)))

        def scores(g):
            for h in range(g * GB, (g + 1) * GB):
                q, k, _ = qkv[h]
                s = jax.lax.dot_general(q, k, NT, preferred_element_type=f32)
                s = jnp.where(mask, s, -1e9)
                p = jnp.exp2(s - jnp.max(s, axis=1, keepdims=True))
                p = p * recip(jnp.sum(p, axis=1, keepdims=True))
                pr[h] = p.astype(bf16)

        def pv(g):
            for h in range(g * GB, (g + 1) * GB):
                ov[h] = jnp.dot(pr[h], qkv[h][2], preferred_element_type=f32).astype(bf16)

        acc = [None] * 8

        def oproj(g4):
            og = jnp.concatenate([ov[h] for h in range(4 * g4, 4 * g4 + 4)], axis=1)
            for j in range(8):
                a = jnp.dot(og, unpack(bo_v[j + z, g4 * 256:(g4 + 1) * 256, :]),
                            preferred_element_type=f32)
                acc[j] = a if acc[j] is None else a + acc[j]

        for t in range(NGB):
            proj(t)
            if t >= 1:
                scores(t - 1)
            if t >= 2:
                pv(t - 2)
        oproj(0)
        scores(NGB - 1)
        oproj(1)
        pv(NGB - 2)
        oproj(2)
        oproj(3)
        pv(NGB - 1)
        for g4 in range(4, 8):
            oproj(g4)
        return jnp.concatenate(acc, axis=1)

    def b_body(j, carry):
        base = pl.multiple_of(j * 64, 64)
        xa = x_v[pl.ds(base, 32), :]
        xb = x_v[pl.ds(base + 32, 32), :]
        xb32 = xb.astype(f32)
        saved = {}
        zero8 = jnp.zeros((8, 128), f32)

        lhs_a = jnp.concatenate(
            [xa, jnp.concatenate([mem_v[...], xb32[0:8]], axis=0).astype(bf16)], axis=0)

        def operands_a(h, q, k, v):
            q = q * CB
            ka = jnp.concatenate([k[32:40], k[0:32], zero8], axis=0).astype(bf16)
            va = jnp.concatenate([v[32:40], v[0:32], zero8], axis=0).astype(bf16)
            saved[h] = (q[24:32], q[40:48], k[40:48], v[40:48], ka, va)
            return jnp.concatenate([q[32:40], q[0:24]], axis=0).astype(bf16), ka, va

        acc_a = step(lhs_a, operands_a, mask_a, 0)

        oa = jnp.concatenate([unpack(o_v[g, pl.ds(half(base), 32), :]) for g in range(8)], axis=1)
        a_out = jnp.concatenate(
            [jnp.dot(oa[:, 128:], unpack(wo_v[c, 64:, :]), preferred_element_type=f32)
             + s0[pl.ds(base, 64), c * 128:(c + 1) * 128] for c in range(4)]
            + [jnp.dot(oa, unpack(wo_v[c]), preferred_element_type=f32) for c in range(4, 8)], axis=1)

        lhs_b = jnp.concatenate(
            [xb[16:32], jnp.concatenate([acc_a[0:8], xb32[8:16]], axis=0).astype(bf16)], axis=0)

        def operands_b(h, q, k, v):
            q = q * CB
            qa_tail, q0, k0, v0, ka, va = saved[h]
            qb = jnp.concatenate([q[16:24], q0, q[24:32], q[0:16], qa_tail], axis=0).astype(bf16)
            kb = jnp.concatenate([k[16:24], k0, k[24:32], k[0:16], zero8], axis=0).astype(bf16)
            vb = jnp.concatenate([v[16:24], v0, v[24:32], v[0:16], zero8], axis=0).astype(bf16)
            return qb, jnp.concatenate([kb, ka], axis=0), jnp.concatenate([vb, va], axis=0)

        acc_b = step(lhs_b, operands_b, mask_b, z_ref[0])
        mem_v[...] = acc_b[0:8]

        b_out = jnp.concatenate([acc_a[8:32], acc_b[40:48], acc_b[8:40]], axis=0)
        x32 = jnp.concatenate([xa.astype(f32), xb32], axis=0)
        g = jax.nn.sigmoid(jnp.sum(x32 * gate, axis=1, keepdims=True))
        out_v[pl.ds(base, 64), :] = (g * a_out + (1.0 - g) * b_out).astype(bf16)
        pltpu.make_async_copy(out_v.at[pl.ds(base, 64)], out_hbm.at[pl.ds(base, 64)], sem_o).start()
        return carry

    jax.lax.fori_loop(0, S // 64, b_body, 0)
    pltpu.make_async_copy(out_v, out_hbm, sem_o).wait()


@functools.partial(jax.jit, static_argnames=("B_seg_len",))
def pallas_gated_mix__grouped_kv_mqa__memory_aug_recurrent_mem_tr__prompt_kernel(
    A_x, A_wq, A_wk, A_wv, A_wo, B_x, B_mem0, B_Wq, B_Wk, B_Wv, B_Wo, B_seg_len, gate_w,
):
    del B_x
    assert B_seg_len == SEG
    assert A_x.shape == (1, S, D) and B_Wq.shape == (D, H, DHB) and B_mem0.shape == (1, M, D)
    out = pl.pallas_call(
        _kernel,
        out_shape=jax.ShapeDtypeStruct((S, D), bf16),
        in_specs=[pl.BlockSpec(memory_space=pl.ANY)] * 11,
        out_specs=pl.BlockSpec(memory_space=pl.ANY),
        scratch_shapes=[
            pltpu.VMEM((2 * DHA, D), bf16),
            pltpu.VMEM((M, D), bf16),
            pltpu.VMEM((D,), bf16),
            pltpu.VMEM((S, D), bf16),
            pltpu.VMEM((4, D, 256), bf16),
            pltpu.VMEM((8, D, 128), bf16),
            pltpu.VMEM((8, D // 2, 128), u32),
            pltpu.VMEM((3, D, H, DHB), bf16),
            pltpu.VMEM((3, H, D // 2, DHB), u32),
            pltpu.VMEM((8, H * DHB, 128), bf16),
            pltpu.VMEM((8, H * DHB // 2, 128), u32),
            pltpu.VMEM((9, 64, S), u32),
            pltpu.VMEM((8, XR, 128), f32),
            pltpu.VMEM((XR, 128), f32),
            pltpu.VMEM((DHA, S), f32),
            pltpu.VMEM((5, S // 2, 128), u32),
            pltpu.VMEM((8, S // 2, 128), u32),
            pltpu.VMEM((DHA // 2, S), u32),
            pltpu.VMEM((S, QB), f32),
            pltpu.VMEM((S, QB), f32),
            pltpu.VMEM((S, QB), f32),
            pltpu.VMEM((S, QB), f32),
            pltpu.VMEM((128, QB), f32),
            pltpu.VMEM((8, QB), f32),
            pltpu.VMEM((8, QB), f32),
            pltpu.VMEM((32, QB), f32),
            pltpu.VMEM((M, D), f32),
            pltpu.VMEM((S, D), bf16),
            pltpu.SMEM((3,), jnp.int32),
            pltpu.SemaphoreType.DMA((5,)),
            pltpu.SemaphoreType.DMA((4,)),
            pltpu.SemaphoreType.DMA((WCH,)),
            pltpu.SemaphoreType.DMA((2,)),
            pltpu.SemaphoreType.DMA,
        ],
        compiler_params=pltpu.CompilerParams(vmem_limit_bytes=120 * 1024 * 1024),
    )(
        A_x.reshape(S, D), A_wq, A_wk.T, A_wv.T, A_wo, B_mem0.reshape(M, D),
        B_Wq, B_Wk, B_Wv, B_Wo.reshape(H * DHB, D), gate_w,
    )
    return out.reshape(1, S, D)
```

```python
import functools

import jax
import jax.numpy as jnp
import jax.experimental.pallas as pl
import jax.experimental.pallas.tpu as pltpu

bf16 = jnp.bfloat16
f32 = jnp.float32
u32 = jnp.uint32

S = 2048
D = 1024
H = 32
DHA = 32
DHB = 128
M = 8
SEG = 32
L = M + SEG
LP = 48
LOG2E = 1.4426950408889634
CA = DHA ** -0.5 * LOG2E
CB = DHB ** -0.5 * LOG2E

XR = 512
HX = XR // 2
QB = 512
CK = 128
NC = S // CK
NGA = (S // QB) * 8
AU = 2
LAG = 2
PACE = 2
WCH = 8
WR = D // WCH
GB = 2
NGB = H // GB

NT = (((1,), (1,)), ((), ()))


def pack(v):
    return pltpu.bitcast(v.astype(bf16), u32)


def unpack(w):
    return pltpu.bitcast(w, bf16)


def half(r0):
    return r0 // 2 if isinstance(r0, int) else pl.multiple_of(jax.lax.shift_right_logical(r0, 1), 8)


def recip(l):
    r = pl.reciprocal(l, approx=True)
    return r * (2.0 - l * r)


def zero_after(v):
    return (pltpu.bitcast(v, u32) >> 31) >> 1


def _kernel(x_hbm, wq_hbm, wkt_hbm, wvt_hbm, wo_hbm, mem0_hbm, bq_hbm, bk_hbm, bv_hbm, bo_hbm, gate_hbm,
            out_hbm,
            wkv_v, mem0_v, gate_v, x_v, wq_v, wos_v, wo_v, stage_v, w_v, bos_v, bo_v,
            q_v, qn_v, q7_v, kt_v, kp_v, o_v, vt_v, s0, s1, s2, s3, ot_v, mx_v, m3_v, l_v,
            mem_v, out_v, z_ref, sem_x, sem_w, sem_b, sem_s, sem_o):
    def cp_x(r0, n, k):
        return pltpu.make_async_copy(x_hbm.at[pl.ds(r0, n)], x_v.at[pl.ds(r0, n)], sem_x.at[k])

    def cp_wq(k):
        col = k * 256 if isinstance(k, int) else pl.multiple_of(k * 256, 256)
        return pltpu.make_async_copy(wq_hbm.at[:, pl.ds(col, 256)], wq_v.at[k], sem_w.at[k])

    def cp_b(c):
        r0 = pl.multiple_of(c * WR, WR)
        col = pl.multiple_of(c * 128, 128)
        cps = [pltpu.make_async_copy(src.at[pl.ds(r0, WR)], stage_v.at[t, pl.ds(r0, WR)], sem_b.at[c])
               for t, src in enumerate((bq_hbm, bk_hbm, bv_hbm))]
        cps.append(pltpu.make_async_copy(bo_hbm.at[:, pl.ds(col, 128)], bos_v.at[c], sem_b.at[c]))
        cps.append(pltpu.make_async_copy(wo_hbm.at[:, pl.ds(col, 128)], wos_v.at[c], sem_b.at[c]))
        return cps

    cp_kv = [pltpu.make_async_copy(src, wkv_v.at[pl.ds(i * DHA, DHA)], sem_s.at[0])
             for i, src in enumerate((wkt_hbm, wvt_hbm))]
    cp_late = [pltpu.make_async_copy(mem0_hbm, mem0_v, sem_s.at[1]),
               pltpu.make_async_copy(gate_hbm, gate_v, sem_s.at[1])]
    issue = [cp_kv + [cp_x(0, HX, 0)], [cp_wq(0)], [cp_wq(1)], [cp_x(HX, HX, 1)]]

    def start(cps):
        for c in cps:
            c.start()

    def issue_body(i, carry):
        for k, group in enumerate(issue):
            pl.when(i == k)(functools.partial(start, group))
        return carry

    jax.lax.fori_loop(0, len(issue), issue_body, 0)

    for i in range(4 * AU):
        z_ref[i] = 0

    def kv_dot(r0, n):
        kvt = jax.lax.dot_general(wkv_v[...], x_v[pl.ds(r0, n), :], NT, preferred_element_type=f32)
        vt_v[:, pl.ds(r0, n)] = pack(kvt[DHA:])
        kt_v[:, pl.ds(r0, n)] = kvt[:DHA]

    def k_pad(r0, n):
        kt = jnp.concatenate([kt_v[:, pl.ds(r0, n)], jnp.zeros((128 - DHA, n), f32)], axis=0)
        kp_v[0, pl.ds(half(r0), n // 2), :] = pack(kt.T)

    def q_dot(r0, n, k, gg):
        w = wq_v[k, :, gg * 128:(gg + 1) * 128]
        return jnp.dot(x_v[pl.ds(r0, n), :], w, preferred_element_type=f32) * CA

    def q_early(r0, n, k):
        for gg in range(2):
            qn_v[2 * k + gg, pl.ds(r0, n), :] = q_dot(r0, n, k, gg)

    for c in cp_kv:
        c.wait()
    cp_x(0, HX, 0).wait()
    start([cp_wq(2), cp_wq(3)])
    kv_dot(0, HX)

    def early_a(k, carry):
        cp_wq(k).wait()
        cp_x(pl.multiple_of(XR + k * XR, XR), XR, 2 + k).start()
        q_early(0, HX, k)
        return carry

    jax.lax.fori_loop(0, 2, early_a, 0)
    cp_x(HX, HX, 1).wait()
    start([cp_x(3 * XR, XR, 4)])
    kv_dot(HX, HX)
    q_early(HX, HX, 0)
    q_early(HX, HX, 1)
    start(cp_b(0) + cp_late)

    def early_b(k, carry):
        cp_wq(k).wait()
        q_early(0, XR, k)
        return carry

    jax.lax.fori_loop(2, 4, early_b, 0)
    q7_v[...] = jnp.zeros_like(q7_v)

    def a_proj(i, carry):
        r0 = pl.multiple_of(i * XR, XR)
        cp_x(r0, XR, 1 + i).wait()
        kv_dot(r0, XR)
        for g in range(8):
            qg = q_dot(r0, XR, g // 2, g % 2)
            if g < 7:
                q_v[g, :, pl.ds(r0, XR)] = pack(qg.T)
            else:
                q7_v[...] = qg
            if g == 0:
                q_v[7, :, pl.ds(pl.multiple_of(jnp.maximum(r0 - XR, XR), XR), XR)] = pack(q7_v[...].T)
            if 1 <= g <= 3:
                gl = jnp.minimum(3 * (i - 1) + g - 1, 7)
                q_v[gl, :, 0:XR] = pack(qn_v[gl].T)
            if g == 4:
                k_pad(pl.multiple_of(r0 - XR, XR), XR)
            if g == 5:
                k_pad(r0, XR)
        return carry

    jax.lax.fori_loop(1, S // XR, a_proj, 0)
    q_v[7, :, S - XR:] = pack(q7_v[...].T)
    for c in range(1, WCH):
        start(cp_b(c))

    bufs = (s0, s1, s2, s3)
    mid = []

    def load_q(it, last=False):
        qb = jnp.where(last, 0, jax.lax.shift_right_logical(it, 3))
        g = jnp.where(last, 8, it & 7)
        return unpack(q_v[g, :, pl.ds(pl.multiple_of(qb * QB, QB), QB)])

    def p1chunk(qg, j, c, mx, z, zk=0, full=False):
        k = unpack(kp_v[zk, c * CK // 2:(c + 1) * CK // 2, :])
        if full:
            s = jnp.dot(k, qg, preferred_element_type=f32)
        else:
            s = jnp.dot(k[:, 0:DHA], qg[j * DHA:(j + 1) * DHA], preferred_element_type=f32)
        bufs[j][pl.ds(pl.multiple_of(z + c * CK, 8), CK), :] = s
        mid.append(s[64:72, QB - 128:])
        sm = jnp.max(s.reshape(CK // 8, 8, QB), axis=0)
        return sm if mx is None else jnp.maximum(mx, sm)

    def p2chunk(j, m, c, l, o, z):
        sc = bufs[j][pl.ds(pl.multiple_of(z + c * CK, 8), CK), :].reshape(CK // 8, 8, QB)
        p = jnp.exp2(sc - m[None])
        t = p
        while t.shape[0] > 1:
            t4 = t.reshape(t.shape[0] // 2, 2, 8, QB)
            t = t4[:, 0] + t4[:, 1]
        ls = t[0]
        l = ls if l is None else l + ls
        pb = p.reshape(CK, QB).astype(bf16)
        oc = jnp.dot(unpack(vt_v[:, c * CK:(c + 1) * CK]), pb, preferred_element_type=f32)
        return l, (oc if o is None else oc + o)

    def colmax(mx):
        return jnp.broadcast_to(jnp.max(mx, axis=0, keepdims=True), (8, QB))

    def fin(it, l3, o3):
        qb = jax.lax.shift_right_logical(it, 3)
        g = it & 7
        parts = []
        for j in range(4):
            lj = l_v[j * 8:(j + 1) * 8, :] if j < 3 else l3
            oj = ot_v[j * 32:(j + 1) * 32, :] if j < 3 else o3
            parts.append(oj * recip(jnp.sum(lj, axis=0, keepdims=True)))
        ot = jnp.concatenate(parts, axis=0)
        o_v[g, pl.ds(pl.multiple_of(qb * (QB // 2), QB // 2), QB // 2), :] = pack(ot.T)

    def relayout(t, b, hq, pace):
        blk = stage_v[t, pl.ds(pl.multiple_of(b * 16, 16), 16), hq * 8:(hq + 1) * 8, :]
        blk = unpack(pltpu.bitcast(blk, u32) | pace[None, 0:4])
        w_v[t, hq * 8:(hq + 1) * 8, pl.ds(pl.multiple_of(b * 8, 8), 8), :] = pltpu.bitcast(
            jnp.swapaxes(blk, 0, 1), u32)

    def repack(src, dst, c, r0, n, pace):
        w = pltpu.bitcast(src[c, pl.ds(pl.multiple_of(r0, 16), n), :], u32).reshape(n // 16, 8, 128)
        dst[c, pl.ds(half(r0), n // 2), :] = (w | pace[None]).reshape(n // 2, 128)

    ot_v[...] = jnp.zeros_like(ot_v)
    l_v[...] = jnp.ones_like(l_v)
    m3_v[...] = jnp.zeros_like(m3_v)
    s3[(NC - LAG) * CK:, :] = jnp.zeros((LAG * CK, QB), f32)
    qg0 = load_q(0)
    mx0 = None
    for c in range(NC):
        mx0 = p1chunk(qg0, 0, c, mx0, z_ref[0])
    mx_v[...] = mx0

    def a_body(i, carry):
        it0 = i * AU
        zz = [z_ref[n] for n in range(2)]
        zk = [0] + [z_ref[n] for n in range(2, 4 * AU)]
        last = it0 + AU == NGA
        qgs = [load_q(it0 + u) for u in range(AU)] + [load_q(it0 + AU, last)]
        mxs = {0: mx_v[...]}
        ms = {-1: m3_v[...]}
        l = l_v[24:32, :]
        o = ot_v[96:128, :]
        mx = None
        hist = []
        for tt in range(AU * 4 * NC):
            u, t = divmod(tt, 4 * NC)
            it = it0 + u
            j1, c1 = tt // NC + 1, tt % NC
            mx = p1chunk(qgs[j1 // 4], j1 % 4, c1, None if c1 == 0 else mx, zz[0],
                         jnp.where(last, 1, 0) if j1 == 4 * AU else zk[j1 - 1], j1 == 4 * AU)
            hist.append(mx)
            if c1 == NC - 1:
                mxs[j1] = mx
            j2, c2 = divmod(tt - LAG, NC)
            if c2 == 0:
                ms[j2] = colmax(mxs[j2])
                l = o = None
            mm = ms[j2]
            if tt >= PACE:
                mm = pltpu.bitcast(pltpu.bitcast(mm, u32) | zero_after(hist[tt - PACE]), f32)
            l, o = p2chunk(j2 % 4, mm, c2, l, o, zz[1])
            if c2 == NC - 1:
                if j2 % 4 == 3:
                    fin(jnp.maximum(it - 1, 0), l, o)
                else:
                    ot_v[(j2 % 4) * 32:(j2 % 4 + 1) * 32, :] = o
                    l_v[(j2 % 4) * 8:(j2 % 4 + 1) * 8, :] = l
            if 8 <= t < 56:
                pace = zero_after(mid[-2])
                k = (t - 8) // 2
                ch = jax.lax.shift_right_logical(it, 2)
                if t % 2 == 0:
                    relayout(k // 8, it * 2 + (k // 4) % 2, k % 4, pace)
                elif k < 4:
                    repack(bos_v, bo_v, ch, (it & 3) * 1024 + k * 256, 256, pace)
                elif k == 4:
                    repack(wos_v, wo_v, ch, (it & 3) * 256, 256, pace)
        ot_v[96:128, :] = o
        l_v[24:32, :] = l
        m3_v[...] = ms[4 * AU - 1]
        mx_v[...] = mx
        return carry

    def a_outer(ch, carry):
        for c in cp_b(ch):
            c.wait()

        @pl.when(ch == WCH - 1)
        def _():
            kp_v[1] = o_v[0]
            for c in range(4):
                q_v[8, :, c * 128:(c + 1) * 128] = wo_v[c, 0:64, :]

        per = NGA // WCH // AU
        return jax.lax.fori_loop(ch * per, (ch + 1) * per, a_body, carry)

    jax.lax.fori_loop(0, WCH, a_outer, 0)
    l = l_v[24:32, :]
    o = ot_v[96:128, :]
    for c in range(NC - LAG, NC):
        l, o = p2chunk(3, m3_v[...], c, l, o, z_ref[1])
    fin(NGA - 1, l, o)

    qq = jax.lax.broadcasted_iota(jnp.int32, (32, LP), 0)
    kk = jax.lax.broadcasted_iota(jnp.int32, (32, LP), 1)
    mask_a = kk <= jnp.where(qq < M, L - 1, qq)
    qq = jax.lax.broadcasted_iota(jnp.int32, (LP, 2 * LP), 0)
    kk = jax.lax.broadcasted_iota(jnp.int32, (LP, 2 * LP), 1)
    lo = jnp.where(qq < L, 0, LP)
    hi = jnp.where(qq < M, L - 1, jnp.where(qq < L, qq, qq - M + LP))
    mask_b = (kk >= lo) & (kk <= hi)
    for c in cp_late:
        c.wait()
    gate = gate_v[...].astype(f32).reshape(1, D)
    mem_v[...] = mem0_v[...].astype(f32)

    def step(lhs, operands, mask, z):
        qkv, pr, ov = {}, {}, {}

        def proj(g):
            for h in range(g * GB, (g + 1) * GB):
                qkv[h] = operands(h, *(jnp.dot(lhs, unpack(w_v[t + z, h]), preferred_element_type=f32)
                                       for t in range(3)))

        def scores(g):
            for h in range(g * GB, (g + 1) * GB):
                q, k, _ = qkv[h]
                s = jax.lax.dot_general(q, k, NT, preferred_element_type=f32)
                s = jnp.where(mask, s, -1e9)
                p = jnp.exp2(s - jnp.max(s, axis=1, keepdims=True))
                p = p * recip(jnp.sum(p, axis=1, keepdims=True))
                pr[h] = p.astype(bf16)

        def pv(g):
            for h in range(g * GB, (g + 1) * GB):
                ov[h] = jnp.dot(pr[h], qkv[h][2], preferred_element_type=f32).astype(bf16)

        acc = [None] * 8

        def oproj(g4):
            og = jnp.concatenate([ov[h] for h in range(4 * g4, 4 * g4 + 4)], axis=1)
            for j in range(8):
                a = jnp.dot(og, unpack(bo_v[j + z, g4 * 256:(g4 + 1) * 256, :]),
                            preferred_element_type=f32)
                acc[j] = a if acc[j] is None else a + acc[j]

        for t in range(NGB):
            proj(t)
            if t >= 1:
                scores(t - 1)
            if t >= 2:
                pv(t - 2)
        oproj(0)
        scores(NGB - 1)
        oproj(1)
        pv(NGB - 2)
        oproj(2)
        oproj(3)
        pv(NGB - 1)
        for g4 in range(4, 8):
            oproj(g4)
        return jnp.concatenate(acc, axis=1)

    def b_body(j, carry):
        base = pl.multiple_of(j * 64, 64)
        xa = x_v[pl.ds(base, 32), :]
        xb = x_v[pl.ds(base + 32, 32), :]
        xb32 = xb.astype(f32)
        saved = {}
        zero8 = jnp.zeros((8, 128), f32)

        lhs_a = jnp.concatenate(
            [xa, jnp.concatenate([mem_v[...], xb32[0:8]], axis=0).astype(bf16)], axis=0)

        def operands_a(h, q, k, v):
            q = q * CB
            ka = jnp.concatenate([k[32:40], k[0:32], zero8], axis=0).astype(bf16)
            va = jnp.concatenate([v[32:40], v[0:32], zero8], axis=0).astype(bf16)
            saved[h] = (q[24:32], q[40:48], k[40:48], v[40:48], ka, va)
            return jnp.concatenate([q[32:40], q[0:24]], axis=0).astype(bf16), ka, va

        acc_a = step(lhs_a, operands_a, mask_a, 0)

        oa = jnp.concatenate([unpack(o_v[g, pl.ds(half(base), 32), :]) for g in range(8)], axis=1)
        a_out = jnp.concatenate(
            [jnp.dot(oa[:, 128:], unpack(wo_v[c, 64:, :]), preferred_element_type=f32)
             + s0[pl.ds(base, 64), c * 128:(c + 1) * 128] for c in range(4)]
            + [jnp.dot(oa, unpack(wo_v[c]), preferred_element_type=f32) for c in range(4, 8)], axis=1)

        lhs_b = jnp.concatenate(
            [xb[16:32], jnp.concatenate([acc_a[0:8], xb32[8:16]], axis=0).astype(bf16)], axis=0)

        def operands_b(h, q, k, v):
            q = q * CB
            qa_tail, q0, k0, v0, ka, va = saved[h]
            qb = jnp.concatenate([q[16:24], q0, q[24:32], q[0:16], qa_tail], axis=0).astype(bf16)
            kb = jnp.concatenate([k[16:24], k0, k[24:32], k[0:16], zero8], axis=0).astype(bf16)
            vb = jnp.concatenate([v[16:24], v0, v[24:32], v[0:16], zero8], axis=0).astype(bf16)
            return qb, jnp.concatenate([kb, ka], axis=0), jnp.concatenate([vb, va], axis=0)

        acc_b = step(lhs_b, operands_b, mask_b, z_ref[0])
        mem_v[...] = acc_b[0:8]

        b_out = jnp.concatenate([acc_a[8:32], acc_b[40:48], acc_b[8:40]], axis=0)
        x32 = jnp.concatenate([xa.astype(f32), xb32], axis=0)
        g = jax.nn.sigmoid(jnp.sum(x32 * gate, axis=1, keepdims=True))
        out_v[pl.ds(base, 64), :] = (g * a_out + (1.0 - g) * b_out).astype(bf16)
        pltpu.make_async_copy(out_v.at[pl.ds(base, 64)], out_hbm.at[pl.ds(base, 64)], sem_o).start()
        return carry

    jax.lax.fori_loop(0, S // 64, b_body, 0)
    pltpu.make_async_copy(out_v, out_hbm, sem_o).wait()


@jax.jit
def pallas_gated_mix__grouped_kv_mqa__memory_aug_recurrent_mem_tr__prompt_kernel(
    A_x, A_wq, A_wk, A_wv, A_wo, B_x, B_mem0, B_Wq, B_Wk, B_Wv, B_Wo, B_seg_len, gate_w,
):
    del B_x
    del B_seg_len
    assert A_x.shape == (1, S, D) and B_Wq.shape == (D, H, DHB) and B_mem0.shape == (1, M, D)
    out = pl.pallas_call(
        _kernel,
        out_shape=jax.ShapeDtypeStruct((S, D), bf16),
        in_specs=[pl.BlockSpec(memory_space=pl.ANY)] * 11,
        out_specs=pl.BlockSpec(memory_space=pl.ANY),
        scratch_shapes=[
            pltpu.VMEM((2 * DHA, D), bf16),
            pltpu.VMEM((M, D), bf16),
            pltpu.VMEM((D,), bf16),
            pltpu.VMEM((S, D), bf16),
            pltpu.VMEM((4, D, 256), bf16),
            pltpu.VMEM((8, D, 128), bf16),
            pltpu.VMEM((8, D // 2, 128), u32),
            pltpu.VMEM((3, D, H, DHB), bf16),
            pltpu.VMEM((3, H, D // 2, DHB), u32),
            pltpu.VMEM((8, H * DHB, 128), bf16),
            pltpu.VMEM((8, H * DHB // 2, 128), u32),
            pltpu.VMEM((9, 64, S), u32),
            pltpu.VMEM((8, XR, 128), f32),
            pltpu.VMEM((XR, 128), f32),
            pltpu.VMEM((DHA, S), f32),
            pltpu.VMEM((2, S // 2, 128), u32),
            pltpu.VMEM((8, S // 2, 128), u32),
            pltpu.VMEM((DHA // 2, S), u32),
            pltpu.VMEM((S, QB), f32),
            pltpu.VMEM((S, QB), f32),
            pltpu.VMEM((S, QB), f32),
            pltpu.VMEM((S, QB), f32),
            pltpu.VMEM((128, QB), f32),
            pltpu.VMEM((8, QB), f32),
            pltpu.VMEM((8, QB), f32),
            pltpu.VMEM((32, QB), f32),
            pltpu.VMEM((M, D), f32),
            pltpu.VMEM((S, D), bf16),
            pltpu.SMEM((4 * AU,), jnp.int32),
            pltpu.SemaphoreType.DMA((5,)),
            pltpu.SemaphoreType.DMA((4,)),
            pltpu.SemaphoreType.DMA((WCH,)),
            pltpu.SemaphoreType.DMA((2,)),
            pltpu.SemaphoreType.DMA,
        ],
        compiler_params=pltpu.CompilerParams(vmem_limit_bytes=120 * 1024 * 1024),
    )(
        A_x.reshape(S, D), A_wq, A_wk.T, A_wv.T, A_wo, B_mem0.reshape(M, D),
        B_Wq, B_Wk, B_Wv, B_Wo.reshape(H * DHB, D), gate_w,
    )
    return out.reshape(1, S, D)
```
